```python
import jax
import jax.numpy as jnp

def _softmax(x, axis=-1):
    return jax.nn.softmax(x, axis=axis)

def _gelu(x):
    return jax.nn.gelu(x, approximate=True)

def _silu(x):
    return jax.nn.silu(x)

def _sigmoid(x):
    return jax.nn.sigmoid(x)

def _layernorm(x, axis=-1, eps=1e-05):
    m = jnp.mean(x, axis=axis, keepdims=True)
    v = jnp.var(x, axis=axis, keepdims=True)
    return (x - m) / jnp.sqrt(v + eps)

def _scatter_add(tgt, idx, src, axis=0):
    return tgt.at[idx].add(src)

def _segment_sum(src, seg, n):
    return jax.ops.segment_sum(src, seg, n)

class _Rng:

    def __init__(self, key):
        self._k = key

    def _next(self):
        self._k, sub = jax.random.split(self._k)
        return sub

    def normal(self, shape):
        return jax.random.normal(self._next(), shape, dtype=jnp.bfloat16)

    def randint(self, lo, hi, shape):
        return jax.random.randint(self._next(), shape, lo, hi, dtype=jnp.int32)

    def uniform(self, shape, lo=0.0, hi=1.0):
        return jax.random.uniform(self._next(), shape, jnp.bfloat16, lo, hi)

    def permutation(self, n):
        return jax.random.permutation(self._next(), n)
kernel_name = 'adaLN_cond__compressed_kv_cla__dense_activation_relu__decode'

def setup_inputs():
    _rng = _Rng(jax.random.key(int.from_bytes(__import__("os").urandom(4), "little")))
    _w = lambda a: (lambda t: t.astype(jnp.bfloat16) if jnp.issubdtype(t.dtype, jnp.floating) else t)(jnp.asarray(a))

    def _A_setup():
        B, H, Sq, Sk, D, M = (8, 32, 1, 4096, 128, 512)
        Dc = 4 * D
        return {'x': _w((lambda *s: _rng.normal(s) * 0.05)(B, Sq, M)), 'c_kv': _w((lambda *s: _rng.normal(s) * 0.05)(B, Sk, Dc)), 'w_q': _w((lambda *s: _rng.normal(s) * 0.05)(M, H, D) * M ** (-0.5)), 'w_uk': _w((lambda *s: _rng.normal(s) * 0.05)(Dc, H, D) * Dc ** (-0.5)), 'w_uv': _w((lambda *s: _rng.normal(s) * 0.05)(Dc, H, D) * Dc ** (-0.5)), 'w_o': _w((lambda *s: _rng.normal(s) * 0.05)(H, D, M) * (H * D) ** (-0.5))}
    _A_in = _A_setup()

    def _B_setup():
        B, S, D, Dff = (8, 1, 512, 1792)
        return {'x': _w((lambda *s: _rng.normal(s) * 0.05)(B, S, D)), 'w1': _w((lambda *s: _rng.normal(s) * 0.05)(D, Dff)), 'w2': _w((lambda *s: _rng.normal(s) * 0.05)(Dff, D))}
    _B_in = _B_setup()
    return {'A_x': _A_in['x'], 'A_c_kv': _A_in['c_kv'], 'A_w_q': _A_in['w_q'], 'A_w_uk': _A_in['w_uk'], 'A_w_uv': _A_in['w_uv'], 'A_w_o': _A_in['w_o'], 'B_x': _B_in['x'], 'B_w1': _B_in['w1'], 'B_w2': _B_in['w2'], 'c': _w((lambda *s: _rng.normal(s) * 0.05)(8, 512)), 'w_mod': _w((lambda *s: _rng.normal(s) * 0.05)(512, 6 * 512) * 512 ** (-0.5))}

def reference(A_x, A_c_kv, A_w_q, A_w_uk, A_w_uv, A_w_o, B_x, B_w1, B_w2, c, w_mod):

    def _A_ref(x, c_kv, w_q, w_uk, w_uv, w_o):
        B, Sq, M = (x.shape[0], x.shape[1], x.shape[2])
        Sk = c_kv.shape[1]
        H, D = (w_q.shape[1], w_q.shape[2])
        q = jnp.einsum('bqm,mhd->bhqd', x, w_q)
        k = jnp.einsum('bkc,chd->bhkd', c_kv, w_uk)
        v = jnp.einsum('bkc,chd->bhkd', c_kv, w_uv)
        scores = jnp.einsum('bhqd,bhkd->bhqk', q, k) * D ** (-0.5)
        off = Sk - Sq
        qi = jnp.arange(Sq)[:, None]
        kj = jnp.arange(Sk)[None, :]
        cmask = kj <= qi + off
        scores = jnp.where(cmask[None, None], scores, -1000000000.0)
        p = _softmax(scores, axis=-1)
        ctx = jnp.einsum('bhqk,bhkd->bhqd', p, v)
        return jnp.einsum('bhqd,hdm->bqm', ctx, w_o)

    def _B_ref(x, w1, w2):
        h = jnp.einsum('bsd,df->bsf', x, w1)
        zero = jnp.zeros_like(h)
        h = jnp.maximum(h, zero)
        return jnp.einsum('bsf,fd->bsd', h, w2)
    x = A_x
    mod = (_silu(c) @ w_mod).reshape(c.shape[0], 6, 1, -1)
    sa, ca, ga, sb, cb, gb = (mod[:, 0].copy(), mod[:, 1].copy(), mod[:, 2].copy(), mod[:, 3].copy(), mod[:, 4].copy(), mod[:, 5].copy())
    h = _layernorm(x, axis=-1) * (1 + ca) + sa
    x = x + ga * _A_ref(h, A_c_kv, A_w_q, A_w_uk, A_w_uv, A_w_o)
    h = _layernorm(x, axis=-1) * (1 + cb) + sb
    x = x + gb * _B_ref(h, B_w1, B_w2)
    return x
```

```python
import functools
import jax
import jax.numpy as jnp
from jax import lax
import jax.experimental.pallas as pl
import jax.experimental.pallas.tpu as pltpu

B, H, SK, D, M, DC, DFF = 8, 32, 4096, 128, 512, 512, 1792
F32, BF16, U32 = jnp.float32, jnp.bfloat16, jnp.uint32
NT = (((1,), (1,)), ((), ()))


def _ln(x):
    m = jnp.mean(x, axis=-1, keepdims=True)
    xc = x - m
    v = jnp.mean(xc * xc, axis=-1, keepdims=True)
    return xc * lax.rsqrt(v + 1e-5)


def _mm(a, b):
    return jnp.dot(a, b, preferred_element_type=F32)


def _head_pair(w_ref, r0, n, j):
    w32 = w_ref.bitcast(U32)
    a = w32[pl.ds(r0 * 16 + j, n // 2, stride=32), :]
    b = w32[pl.ds(r0 * 16 + 16 + j, n // 2, stride=32), :]
    even = (a & 0xFFFF) | (b << 16)
    odd = (a >> 16) | (b & jnp.uint32(0xFFFF0000))
    return pltpu.bitcast(even, BF16), pltpu.bitcast(odd, BF16)


def make(nq=2, nuk=2, nuv=2, no=2, fchunks=(512, 512, 512, 256), ahead=99, nodma=False, extra=None, kc=4096):
    nkc = SK // kc
    def kern(x_h, ckv_h, wq_h, wuk_h, wuv_h, wo_h, w1_h, w2_h, c_h, wm_h, o_ref,
             xb, cb_, ckv, wq, wuk, wuv, wo, w1, w2, wm, qs, os_, sems, ksems):
        cps = []
        def add(src, dst):
            cps.append(pltpu.make_async_copy(src, dst, sems.at[len(cps)]))
            return cps[-1]
        def rows(src, dst, n, tot):
            s = tot // n
            return [add(src.at[pl.ds(i * s, s)], dst.at[pl.ds(i * s, s)]) for i in range(n)]
        c_cp = add(c_h, cb_)
        x_cp = add(x_h, xb)
        wm0 = add(wm_h.at[:, pl.ds(0, 2 * M)], wm.at[:, pl.ds(0, 2 * M)])
        wq_cp = rows(wq_h, wq, nq, M * H)
        wuk_cp = rows(wuk_h, wuk, nuk, DC * H)
        npre = len(cps)
        wm1 = add(wm_h.at[:, pl.ds(2 * M, 4 * M)], wm.at[:, pl.ds(2 * M, 4 * M)])
        wuv_cp = rows(wuv_h, wuv, nuv, DC * H)
        wo_cp = rows(wo_h, wo, no, H * D)
        f_cp = []
        f0 = 0
        for fc in fchunks:
            a = add(w1_h.at[:, pl.ds(f0, fc)], w1.at[:, pl.ds(f0, fc)])
            b = add(w2_h.at[pl.ds(f0, fc)], w2.at[pl.ds(f0, fc)])
            f_cp.append((f0, fc, a, b))
            f0 += fc
        kv_cp = lambda b, i: pltpu.make_async_copy(ckv_h.at[b, pl.ds(i * kc, kc)], ckv.at[b, pl.ds(i * kc, kc)], ksems.at[b * nkc + i])
        wait = (lambda cp: None) if nodma else (lambda cp: cp.wait())
        if not nodma:
            for cp in cps[:npre]: cp.start()
            for b in range(min(B, ahead)):
                for i in range(nkc): kv_cp(b, i).start()
            if ahead >= B:
                for cp in cps[npre:]: cp.start()

        wait(c_cp); wait(x_cp)
        cc = cb_[...].astype(F32)
        sc = (cc * jax.nn.sigmoid(cc)).astype(BF16)
        x = xb[...].astype(F32)
        xn = _ln(x)
        wait(wm0)
        mod0 = _mm(sc, wm[:, 0:2 * M])
        h = (xn * (1.0 + mod0[:, M:2 * M]) + mod0[:, 0:M]).astype(BF16)

        s = M // nq
        q = None
        for i in range(nq):
            wait(wq_cp[i])
            w = jnp.concatenate([p for j in range(H // 2) for p in _head_pair(wq, i * s, s, j)], axis=1)
            t = _mm(h[:, i * s:(i + 1) * s], w)
            q = t if q is None else q + t
        q = q.astype(BF16)
        s = DC // nuk
        for i in range(nuk):
            wait(wuk_cp[i])
            for j in range(H // 2):
                for e, w in enumerate(_head_pair(wuk, i * s, s, j)):
                    hh = 2 * j + e
                    r = lax.dot_general(q[:, hh * D:(hh + 1) * D], w, NT, preferred_element_type=F32)
                    for t in range(s // 128):
                        qs[i * (s // 128) + t, hh * B:(hh + 1) * B, :] = r[:, t * 128:(t + 1) * 128]

        def body(b, carry):
            qb = jnp.concatenate([qs[t, pl.ds(b, H, stride=B), :] for t in range(4)], axis=1).astype(BF16)
            ss = []
            for i in range(nkc):
                wait(kv_cp(b, i))
                ss.append(lax.dot_general(qb, ckv[b, i * kc:(i + 1) * kc, :], NT, preferred_element_type=F32))
            if not nodma and ahead < B:
                @pl.when(b + ahead < B)
                def _():
                    for i in range(nkc): kv_cp(b + ahead, i).start()
                @pl.when(b + ahead == B)
                def _():
                    for cp in cps[npre:]: cp.start()
            sc_ = jnp.concatenate(ss, axis=1) * (D ** -0.5)
            mx = jnp.max(sc_, axis=-1, keepdims=True)
            p = jnp.exp(sc_ - mx)
            l = jnp.sum(p, axis=-1, keepdims=True)
            o = _mm(p.astype(BF16), ckv[b]) * (1.0 / l)
            for t in range(4):
                os_[t, pl.ds(b, H, stride=B), :] = o[:, t * 128:(t + 1) * 128]
            return carry
        lax.fori_loop(0, B, body, 0)

        wait(wm1)
        mod1 = _mm(sc, wm[:, 2 * M:6 * M])
        ga, sb, cb, gb = (mod1[:, i * M:(i + 1) * M] for i in range(4))
        s = DC // nuv
        ctx = [None] * H
        for i in range(nuv):
            wait(wuv_cp[i])
            for j in range(H // 2):
                for e, w in enumerate(_head_pair(wuv, i * s, s, j)):
                    hh = 2 * j + e
                    a = jnp.concatenate([os_[i * (s // 128) + t, hh * B:(hh + 1) * B, :] for t in range(s // 128)], axis=1).astype(BF16)
                    t = _mm(a, w)
                    ctx[hh] = t if ctx[hh] is None else ctx[hh] + t
        ctx = jnp.concatenate(ctx, axis=1).astype(BF16)
        s = H * D // no
        ao = None
        for i in range(no):
            wait(wo_cp[i])
            t = _mm(ctx[:, i * s:(i + 1) * s], wo[i * s:(i + 1) * s, :])
            ao = t if ao is None else ao + t
        x1 = x + ga * ao
        h2 = (_ln(x1) * (1.0 + cb) + sb).astype(BF16)
        y = None
        for f0, fc, a, b in f_cp:
            wait(a)
            u = jnp.maximum(_mm(h2, w1[:, f0:f0 + fc]), 0.0).astype(BF16)
            wait(b)
            t = _mm(u, w2[f0:f0 + fc, :])
            y = t if y is None else y + t
        o_ref[...] = (x1 + gb * y).astype(o_ref.dtype)

    nsem = 4 + nq + nuk + nuv + no + 2 * len(fchunks)
    @jax.jit
    def f(A_x, A_c_kv, A_w_q, A_w_uk, A_w_uv, A_w_o, B_x, B_w1, B_w2, c, w_mod):
        V = pltpu.VMEM
        return pl.pallas_call(
            kern, out_shape=jax.ShapeDtypeStruct((B, M), A_x.dtype),
            in_specs=[pl.BlockSpec(memory_space=pltpu.HBM)] * 10,
            out_specs=pl.BlockSpec(memory_space=pltpu.VMEM),
            scratch_shapes=[V((B, M), BF16), V((B, M), BF16), V((B, SK, DC), BF16), V((M * H, D), BF16), V((DC * H, D), BF16),
                            V((DC * H, D), BF16), V((H * D, M), BF16), V((M, DFF), BF16), V((DFF, M), BF16), V((M, 6 * M), BF16),
                            V((4, H * B, 128), F32), V((4, H * B, 128), F32),
                            pltpu.SemaphoreType.DMA((nsem,)), pltpu.SemaphoreType.DMA((B * nkc,))],
            compiler_params=pltpu.CompilerParams(vmem_limit_bytes=100 * 2**20, **(extra or {})),
        )(A_x.reshape(B, M), A_c_kv, A_w_q.reshape(M * H, D), A_w_uk.reshape(DC * H, D), A_w_uv.reshape(DC * H, D),
          A_w_o.reshape(H * D, M), B_w1, B_w2, c, w_mod).reshape(B, 1, M)
    return f


pallas_adaLN_cond__compressed_kv_cla__dense_activation_relu__decode_kernel = make(ahead=2)
```

```python
import functools
import jax
import jax.numpy as jnp
from jax import lax
import jax.experimental.pallas as pl
import jax.experimental.pallas.tpu as pltpu

B, H, SK, D, M, DC, DFF = 8, 32, 4096, 128, 512, 512, 1792
F32, BF16, U32 = jnp.float32, jnp.bfloat16, jnp.uint32
NT = (((1,), (1,)), ((), ()))


def _ln(x):
    m = jnp.mean(x, axis=-1, keepdims=True)
    xc = x - m
    v = jnp.mean(xc * xc, axis=-1, keepdims=True)
    return xc * lax.rsqrt(v + 1e-5)


def _mm(a, b):
    return jnp.dot(a, b, preferred_element_type=F32)


def _head_pair(w_ref, r0, n, j):
    w32 = w_ref.bitcast(U32)
    a = w32[pl.ds(r0 * 16 + j, n // 2, stride=32), :]
    b = w32[pl.ds(r0 * 16 + 16 + j, n // 2, stride=32), :]
    even = (a & 0xFFFF) | (b << 16)
    odd = (a >> 16) | (b & jnp.uint32(0xFFFF0000))
    return pltpu.bitcast(even, BF16), pltpu.bitcast(odd, BF16)


def make(la=2, w2c=(768, 512, 256, 256), unroll=4, extra=None, pr=(0, 1), nsem=6, scale=1, mode=0, nocomp=False):
    def kern(x_h, ckv_h, wq_h, wuk_h, wuv_h, wo_h, w1_h, w2_h, c_h, wm_h, o_ref,
             xb, cb_, ckv, wq, wuk, wuv, wo, w1, w2, wm0, wm1, qs, os_, sems):
        def loop(n, fn):
            u = min(unroll, n)
            def body(i, c):
                for j in range(u): fn(i * u + j)
                return c
            if n // u > 1: lax.fori_loop(0, n // u, body, 0)
            else: body(0, 0)
            for j in range(n // u * u, n): fn(j)

        def row_seg(src, dst, r0, n, piece):
            piece = piece * scale
            def start(sem):
                def one(i):
                    for p in range(2):
                        r = pl.multiple_of(r0 + p * (n // 2) + i * piece, 16)
                        pltpu.make_async_copy(src.at[pl.ds(r, piece)], dst.at[pl.ds(r, piece)], sem).start(priority=pr[p])
                loop(n // 2 // piece, one)
            def wait(sem):
                v = dst.at[pl.ds(r0, n)]
                pltpu.make_async_copy(v, v, sem).wait()
            return start, wait

        def col_seg(src, dst, c0, ncol, pc):
            def start(sem):
                def one(i):
                    for k in range(ncol // pc):
                        for p in range(2):
                            r = pl.multiple_of(p * (M // 2) + i * 16, 16)
                            pltpu.make_async_copy(src.at[pl.ds(r, 16), pl.ds(c0 + k * pc, pc)], dst.at[pl.ds(r, 16), pl.ds(k * pc, pc)], sem).start(priority=pr[p])
                loop(M // 32, one)
            def wait(sem):
                pltpu.make_async_copy(dst, dst, sem).wait()
            return start, wait

        half = M * H // 2
        pre = [col_seg(wm_h, wm0, 0, 2 * M, 2 * M)]
        pre += [row_seg(wq_h, wq, i * half, half, 128) for i in range(2)]
        pre += [row_seg(wuk_h, wuk, i * half, half, 128) for i in range(2)]
        post = [col_seg(wm_h, wm1, 2 * M, 4 * M, 2 * M)]
        post += [row_seg(wuv_h, wuv, i * half, half, 128) for i in range(2)]
        post += [row_seg(wo_h, wo, i * 2048, 2048, 32) for i in range(2)]
        post += [col_seg(w1_h, w1, 0, DFF, DFF // 2)]
        f0 = 0
        for fc in w2c:
            post.append(row_seg(w2_h, w2, f0, fc, 32)); f0 += fc
        NP, NK = len(pre), 2 * B
        kv_seg = lambda k: row_seg(ckv_h, ckv, k * 2048, 2048, 32)
        seg = lambda g: pre[g] if g < NP else (kv_seg(g - NP) if g < NP + NK else post[g - NP - NK])
        ntot = NP + NK + len(post)
        sem = lambda g: sems.at[g % nsem]
        def start(g):
            if g < ntot: seg(g)[0](sem(g))
        def wait(g): seg(g)[1](sem(g))
        G1 = NP + NK
        GW2 = G1 + 6
        def step(g):
            if g + la < GW2: start(g + la)
            elif g + la == GW2:
                for k in range(GW2, ntot): start(k)
            wait(g)

        c_cp = pltpu.make_async_copy(c_h, cb_, sems.at[nsem - 1])
        x_cp = pltpu.make_async_copy(x_h, xb, sems.at[nsem - 1])
        c_cp.start(); x_cp.start()
        for g in range(la): start(g)
        c_cp.wait(); x_cp.wait()
        if nocomp:
            for g in range(ntot): step(g)
            o_ref[...] = w2[0:8, :]
            return
        cc = cb_[...].astype(F32)
        sc = (cc * jax.nn.sigmoid(cc)).astype(BF16)
        x = xb[...].astype(F32)
        xn = _ln(x)
        step(0)
        mod0 = _mm(sc, wm0[...])
        h = (xn * (1.0 + mod0[:, M:2 * M]) + mod0[:, 0:M]).astype(BF16)
        s = M // 2
        q = None
        for i in range(2):
            step(1 + i)
            w = jnp.concatenate([p for j in range(H // 2) for p in _head_pair(wq, i * s, s, j)], axis=1)
            t = _mm(h[:, i * s:(i + 1) * s], w)
            q = t if q is None else q + t
        q = q.astype(BF16)
        for i in range(2):
            step(3 + i)
            for j in range(H // 2):
                for e, w in enumerate(_head_pair(wuk, i * s, s, j)):
                    hh = 2 * j + e
                    r = lax.dot_general(q[:, hh * D:(hh + 1) * D], w, NT, preferred_element_type=F32)
                    for t in range(2):
                        qs[i * 2 + t, hh * B:(hh + 1) * B, :] = r[:, t * 128:(t + 1) * 128]

        def dyn_start(k):
            @pl.when(k < NK)
            def _():
                kv_seg(k)[0](sems.at[(NP + k) % nsem])
            for j in range(la):
                @pl.when(k == NK + j)
                def _():
                    start(G1 + j)
        def dyn_wait(k):
            kv_seg(k)[1](sems.at[(NP + k) % nsem])

        def body(b, carry):
            r0 = pl.multiple_of(b * SK, SK)
            qb = jnp.concatenate([qs[t, pl.ds(b, H, stride=B), :] for t in range(4)], axis=1).astype(BF16)
            if mode == 0:
                ss = []
                for i in range(2):
                    dyn_start(2 * b + i + la)
                    dyn_wait(2 * b + i)
                    ss.append(lax.dot_general(qb, ckv[pl.ds(r0 + i * 2048, 2048), :], NT, preferred_element_type=F32))
                sc_ = jnp.concatenate(ss, axis=1)
            else:
                dyn_start(2 * b + la)
                dyn_wait(2 * b); dyn_wait(2 * b + 1)
                sc_ = lax.dot_general(qb, ckv[pl.ds(r0, SK), :], NT, preferred_element_type=F32)
                dyn_start(2 * b + 1 + la)
            sc_ = sc_ * (D ** -0.5)
            mx = jnp.max(sc_, axis=-1, keepdims=True)
            p = jnp.exp(sc_ - mx)
            l = jnp.sum(p, axis=-1, keepdims=True)
            o = _mm(p.astype(BF16), ckv[pl.ds(r0, SK), :]) * (1.0 / l)
            for t in range(4):
                os_[t, pl.ds(b, H, stride=B), :] = o[:, t * 128:(t + 1) * 128]
            return carry
        lax.fori_loop(0, B, body, 0)

        step(G1)
        mod1 = _mm(sc, wm1[...])
        ga, sb, cb, gb = (mod1[:, i * M:(i + 1) * M] for i in range(4))
        ctx = [None] * H
        for i in range(2):
            step(G1 + 1 + i)
            for j in range(H // 2):
                for e, w in enumerate(_head_pair(wuv, i * s, s, j)):
                    hh = 2 * j + e
                    a = jnp.concatenate([os_[i * 2 + t, hh * B:(hh + 1) * B, :] for t in range(2)], axis=1).astype(BF16)
                    t = _mm(a, w)
                    ctx[hh] = t if ctx[hh] is None else ctx[hh] + t
        ctx = jnp.concatenate(ctx, axis=1).astype(BF16)
        ao = None
        for i in range(2):
            step(G1 + 3 + i)
            t = _mm(ctx[:, i * 2048:(i + 1) * 2048], wo[i * 2048:(i + 1) * 2048, :])
            ao = t if ao is None else ao + t
        x1 = x + ga * ao
        h2 = (_ln(x1) * (1.0 + cb) + sb).astype(BF16)
        step(G1 + 5)
        u = jnp.maximum(_mm(h2, w1[...]), 0.0).astype(BF16)
        y = None
        f0 = 0
        for i, fc in enumerate(w2c):
            step(GW2 + i)
            t = _mm(u[:, f0:f0 + fc], w2[f0:f0 + fc, :])
            y = t if y is None else y + t
            f0 += fc
        o_ref[...] = (x1 + gb * y).astype(o_ref.dtype)

    assert nsem >= la + len(w2c)
    @jax.jit
    def f(A_x, A_c_kv, A_w_q, A_w_uk, A_w_uv, A_w_o, B_x, B_w1, B_w2, c, w_mod):
        V = pltpu.VMEM
        return pl.pallas_call(
            kern, out_shape=jax.ShapeDtypeStruct((B, M), A_x.dtype),
            in_specs=[pl.BlockSpec(memory_space=pltpu.HBM)] * 10,
            out_specs=pl.BlockSpec(memory_space=pltpu.VMEM),
            scratch_shapes=[V((B, M), BF16), V((B, M), BF16), V((B * SK, DC), BF16), V((M * H, D), BF16), V((DC * H, D), BF16),
                            V((DC * H, D), BF16), V((H * D, M), BF16), V((M, DFF), BF16), V((DFF, M), BF16), V((M, 2 * M), BF16), V((M, 4 * M), BF16),
                            V((4, H * B, 128), F32), V((4, H * B, 128), F32), pltpu.SemaphoreType.DMA((nsem,))],
            compiler_params=pltpu.CompilerParams(vmem_limit_bytes=100 * 2**20, **(extra or {})),
        )(A_x.reshape(B, M), A_c_kv.reshape(B * SK, DC), A_w_q.reshape(M * H, D), A_w_uk.reshape(DC * H, D), A_w_uv.reshape(DC * H, D),
          A_w_o.reshape(H * D, M), B_w1, B_w2, c, w_mod).reshape(B, 1, M)
    return f


pallas_adaLN_cond__compressed_kv_cla__dense_activation_relu__decode_kernel = make()
```

```python
import jax
import jax.numpy as jnp
from jax import lax
import jax.experimental.pallas as pl
import jax.experimental.pallas.tpu as pltpu

B, H, SK, D, M, DC, DFF = 8, 32, 4096, 128, 512, 512, 1792
F32, BF16, U32 = jnp.float32, jnp.bfloat16, jnp.uint32
LANES = 128
TILE = 16
WROWS = 256
KEYS = SK // 2
OROWS = H * D // 2
FHALF = DFF // 2
AHEAD = 3
PIECE_KIB = (48, 48, 32)
W2_ROWS = (768, 512, 384, 128)
NSEM = 8


def _layernorm(x):
    xc = x - jnp.mean(x, axis=-1, keepdims=True)
    var = jnp.mean(xc * xc, axis=-1, keepdims=True)
    return xc * lax.rsqrt(var + 1e-5)


def _mm(a, b):
    return jnp.dot(a, b, preferred_element_type=F32)


def _mm_nt(a, b):
    return lax.dot_general(a, b, (((1,), (1,)), ((), ())), preferred_element_type=F32)


def _per_head(w_ref, words):
    words[...] = pltpu.bitcast(w_ref[...], U32)
    for j in range(H // 2):
        even = words[pl.ds(j, WROWS // 2, stride=H), :]
        odd = words[pl.ds(H // 2 + j, WROWS // 2, stride=H), :]
        yield pltpu.bitcast((even & 0xFFFF) | (odd << 16), BF16)
        yield pltpu.bitcast((even >> 16) | (odd & jnp.uint32(0xFFFF0000)), BF16)


def _start(src, dst, sem, queue):
    pltpu.make_async_copy(src, dst, sem).start(priority=queue)


def _wait_filled(buf, sem):
    pltpu.make_async_copy(buf, buf, sem).wait()


def _start_rows(src, s0, dst, d0, n, sem):
    rows_per_kib = 512 // src.shape[1]
    period = sum(PIECE_KIB) * rows_per_kib

    def step(i, carry):
        off = i * period
        for kib in PIECE_KIB:
            size = kib * rows_per_kib
            for queue, half in ((0, n // 2), (1, 0)):
                s = pl.multiple_of(s0 + half + off, TILE)
                d = pl.multiple_of(d0 + half + off, TILE)
                _start(src.at[pl.ds(s, size)], dst.at[pl.ds(d, size)], sem, queue)
            off += size
        return carry

    lax.fori_loop(0, n // 2 // period, step, 0)


def _start_cols(src, c0, dst, sem):
    rows, cols = dst.shape

    def step(i, carry):
        for c in range(0, cols, 1024):
            for queue, half in ((0, rows // 2), (1, 0)):
                r = pl.ds(pl.multiple_of(half + i * TILE, TILE), TILE)
                _start(src.at[r, pl.ds(c0 + c, 1024)], dst.at[r, pl.ds(c, 1024)], sem, queue)
        return carry

    lax.fori_loop(0, rows // 2 // TILE, step, 0)


def _body(x_hbm, ckv_hbm, wq_hbm, wuk_hbm, wuv_hbm, wo_hbm, w1_hbm, w2_hbm, c_hbm, wmod_hbm,
          out_hbm, x_buf, c_buf, out_buf, ckv, wq0, wq1, wuk0, wuk1, wuv0, wuv1, wo0, wo1,
          w1a, w1b, w2, wmod_a, wmod_b, q_lat, o_lat, words, sems):
    def rows(src, i, dst):
        n = dst.shape[0]
        return dst, lambda sem: _start_rows(src, i * n, dst, 0, n, sem)

    def cols(src, c0, dst):
        return dst, lambda sem: _start_cols(src, c0, dst, sem)

    head = [cols(wmod_hbm, 0, wmod_a), rows(wq_hbm, 0, wq0), rows(wq_hbm, 1, wq1),
            rows(wuk_hbm, 0, wuk0), rows(wuk_hbm, 1, wuk1)]
    tail = [cols(wmod_hbm, 2 * M, wmod_b), rows(wuv_hbm, 0, wuv0), rows(wuv_hbm, 1, wuv1),
            rows(wo_hbm, 0, wo0), rows(wo_hbm, 1, wo1)]
    kv0 = len(head)
    tail0 = kv0 + 2 * B
    ffn0 = tail0 + len(tail)
    w2_starts = [sum(W2_ROWS[:i]) for i in range(len(W2_ROWS))]

    def sem(g):
        return sems.at[g % NSEM]

    def start_kv(k):
        _start_rows(ckv_hbm, k * KEYS, ckv, k * KEYS, KEYS, sem(kv0 + k))

    def start(g):
        if g < kv0:
            head[g][1](sem(g))
        elif g < tail0:
            start_kv(g - kv0)
        elif g < ffn0:
            tail[g - tail0][1](sem(g))

    def start_ffn():
        first = [(w1_hbm.at[pl.ds(r, TILE), pl.ds(i * FHALF, FHALF)], dst.at[pl.ds(r, TILE)], sem(ffn0 + i))
                 for i, dst in enumerate((w1a, w1b)) for r in range(0, M, TILE)]
        second = [(w2_hbm.at[pl.ds(r, 2 * TILE)], w2.at[pl.ds(r, 2 * TILE)], sem(ffn0 + 2 + i))
                  for i, (f0, n) in enumerate(zip(w2_starts, W2_ROWS)) for r in range(f0, f0 + n, 2 * TILE)]
        lead = len(first) - len(second)
        for i, piece in enumerate(first):
            _start(*piece, i % 2 if i < lead else 0)
            if i >= lead:
                _start(*second[i - lead], 1)

    def acquire(g):
        start(g + AHEAD)
        if g == ffn0 - 2:
            start_ffn()
        buf = head[g][0] if g < kv0 else tail[g - tail0][0]
        _wait_filled(buf, sem(g))
        return buf

    small = [pltpu.make_async_copy(c_hbm, c_buf, sems.at[NSEM - 1]),
             pltpu.make_async_copy(x_hbm, x_buf, sems.at[NSEM - 2])]
    for cp in small:
        cp.start()
    for g in range(AHEAD):
        start(g)
    for cp in small:
        cp.wait()
    c = c_buf[...].astype(F32)
    cond = (c * jax.nn.sigmoid(c)).astype(BF16)
    x = x_buf[...].astype(F32)
    x_norm = _layernorm(x)

    mod = _mm(cond, acquire(0)[...])
    h = (x_norm * (1.0 + mod[:, M:]) + mod[:, :M]).astype(BF16)
    q = 0.0
    for i in range(2):
        w = jnp.concatenate(list(_per_head(acquire(1 + i), words)), axis=1)
        q += _mm(h[:, i * WROWS:(i + 1) * WROWS], w)
    q = q.astype(BF16)
    for i in range(2):
        for hd, w in enumerate(_per_head(acquire(3 + i), words)):
            r = _mm_nt(q[:, hd * D:(hd + 1) * D], w)
            for t in range(2):
                q_lat[2 * i + t, hd * B:(hd + 1) * B, :] = r[:, t * LANES:(t + 1) * LANES]

    def attend(b, carry):
        heads = pl.ds(b, H, stride=B)
        qb = jnp.concatenate([q_lat[t, heads, :] for t in range(DC // LANES)], axis=1).astype(BF16)
        scores = []
        for i in range(2):
            k = 2 * b + i
            pl.when(k + AHEAD < 2 * B)(lambda: start_kv(k + AHEAD))
            for j in range((AHEAD + i) % 2, AHEAD, 2):
                pl.when(k + AHEAD == 2 * B + j)(lambda: start(tail0 + j))
            keys = pl.ds(pl.multiple_of(k * KEYS, KEYS), KEYS)
            _wait_filled(ckv.at[keys], sem(kv0 + k))
            scores.append(_mm_nt(qb, ckv[keys, :]))
        s = jnp.concatenate(scores, axis=1) * D ** -0.5
        p = jnp.exp(s - jnp.max(s, axis=-1, keepdims=True))
        denom = jnp.sum(p, axis=-1, keepdims=True)
        o = _mm(p.astype(BF16), ckv[pl.ds(pl.multiple_of(b * SK, SK), SK), :]) / denom
        for t in range(DC // LANES):
            o_lat[t, heads, :] = o[:, t * LANES:(t + 1) * LANES]
        return carry

    lax.fori_loop(0, B, attend, 0)

    mod = _mm(cond, acquire(tail0)[...])
    gate_a, shift_b, scale_b, gate_b = (mod[:, i * M:(i + 1) * M] for i in range(4))
    ctx = [0.0] * H
    for i in range(2):
        for hd, w in enumerate(_per_head(acquire(tail0 + 1 + i), words)):
            a = jnp.concatenate([o_lat[2 * i + t, hd * B:(hd + 1) * B, :] for t in range(2)], axis=1)
            ctx[hd] += _mm(a.astype(BF16), w)
    ctx = jnp.concatenate(ctx, axis=1).astype(BF16)
    attn = 0.0
    for i in range(2):
        attn += _mm(ctx[:, i * OROWS:(i + 1) * OROWS], acquire(tail0 + 3 + i)[...])
    x = x + gate_a * attn

    h = (_layernorm(x) * (1.0 + scale_b) + shift_b).astype(BF16)
    act = []
    y = 0.0
    for i, (f0, n) in enumerate(zip(w2_starts, W2_ROWS)):
        while len(act) * FHALF < f0 + n:
            w1 = (w1a, w1b)[len(act)]
            _wait_filled(w1, sem(ffn0 + len(act)))
            act.append(jnp.maximum(_mm(h, w1[...]), 0.0).astype(BF16))
        _wait_filled(w2.at[pl.ds(f0, n)], sem(ffn0 + 2 + i))
        y += _mm(jnp.concatenate(act, axis=1)[:, f0:f0 + n], w2[f0:f0 + n, :])
    out_buf[...] = (x + gate_b * y).astype(out_buf.dtype)
    out = pltpu.make_async_copy(out_buf, out_hbm, sems.at[0])
    out.start()
    out.wait()


def _kernel(*refs):
    pl.run_scoped(lambda sems: _body(*refs, sems), pltpu.SemaphoreType.DMA((NSEM,)))


@jax.jit
def pallas_adaLN_cond__compressed_kv_cla__dense_activation_relu__decode_kernel(
        A_x, A_c_kv, A_w_q, A_w_uk, A_w_uv, A_w_o, B_x, B_w1, B_w2, c, w_mod):
    del B_x
    vmem = pltpu.VMEM
    scratch = (
        [vmem((B, M), BF16)] * 3
        + [vmem((B * SK, DC), BF16)]
        + [vmem((WROWS * H, D), BF16)] * 6
        + [vmem((OROWS, M), BF16)] * 2
        + [vmem((M, FHALF), BF16)] * 2
        + [vmem((DFF, M), BF16), vmem((M, 2 * M), BF16), vmem((M, 4 * M), BF16)]
        + [vmem((DC // LANES, H * B, LANES), F32)] * 2
        + [vmem((WROWS * H // 2, D), U32)]
    )
    out = pl.pallas_call(
        _kernel,
        out_shape=jax.ShapeDtypeStruct((B, M), A_x.dtype),
        in_specs=[pl.BlockSpec(memory_space=pltpu.HBM)] * 10,
        out_specs=pl.BlockSpec(memory_space=pltpu.HBM),
        scratch_shapes=scratch,
        compiler_params=pltpu.CompilerParams(vmem_limit_bytes=96 * 2**20),
    )(A_x.reshape(B, M), A_c_kv.reshape(B * SK, DC), A_w_q.reshape(M * H, D),
      A_w_uk.reshape(DC * H, D), A_w_uv.reshape(DC * H, D), A_w_o.reshape(H * D, M),
      B_w1, B_w2, c, w_mod)
    return out.reshape(B, 1, M)
```

```python
import jax
import jax.numpy as jnp
import numpy as np
from jax import lax
import jax.experimental.pallas as pl
import jax.experimental.pallas.tpu as pltpu

B, H, SK, D, M, DC, DFF = 8, 32, 4096, 128, 512, 512, 1792
F32, BF16, U32 = jnp.float32, jnp.bfloat16, jnp.uint32
LANES = 128
TILE = 16
PIECE = 16384
ROUNDS = 16
EIGHTHS = (4, 0, 5, 1, 6, 2, 7, 3)
FHALF = DFF // 2
W2_ROWS = 256
W2_CHUNKS = ((0, 512, 1024, 1536), (256,), (768,), (1280,))
NSEM = 8


def _layernorm(x):
    xc = x - jnp.mean(x, axis=-1, keepdims=True)
    var = jnp.mean(xc * xc, axis=-1, keepdims=True)
    return xc * lax.rsqrt(var + 1e-5)


def _mm(a, b):
    return jnp.dot(a, b, preferred_element_type=F32)


def _mm_nt(a, b):
    return lax.dot_general(a, b, (((1,), (1,)), ((), ())), preferred_element_type=F32)


def _per_head(w_ref, t, words):
    words[...] = pltpu.bitcast(w_ref[t * LANES * H:(t + 1) * LANES * H, :], U32)
    for j in range(H // 2):
        even = words[pl.ds(j, LANES // 2, stride=H), :]
        odd = words[pl.ds(H // 2 + j, LANES // 2, stride=H), :]
        yield pltpu.bitcast((even & 0xFFFF) | (odd << 16), BF16)
        yield pltpu.bitcast((even >> 16) | (odd & np.uint32(0xFFFF0000)), BF16)


def _rows(start, n):
    return pl.ds(pl.multiple_of(start, TILE), n)


def _loop(lo, hi, fn):
    if lo < hi:
        lax.fori_loop(lo, hi, lambda i, _: fn(i), None)


def _start(pieces):
    for k, piece in enumerate(pieces):
        pltpu.make_async_copy(*piece).start(priority=k % 2)


def _wait_filled(buf, sem):
    pltpu.make_async_copy(buf, buf, sem).wait()


def _fetch(src, dst, base, sem, lo, hi):
    size = PIECE // src.shape[1]

    def one_round(i, first=False, last=False):
        cuts = []
        for e in EIGHTHS:
            a = 0 if first and e == min(EIGHTHS) else size // 2
            b = size if last and e == max(EIGHTHS) else size + size // 2
            cuts.append(_rows(base + (e * ROUNDS + i) * size + a, b - a))
        _start([(src.at[r], dst.at[r], sem) for r in cuts])

    if lo == 0:
        one_round(0, first=True)
    _loop(max(lo, 1), min(hi, ROUNDS - 1), one_round)
    if hi == ROUNDS:
        one_round(ROUNDS - 1, last=True)


def _body(x_hbm, ckv_hbm, wq_hbm, wuk_hbm, wuv_hbm, wo_hbm, w1_hbm, w2_hbm, c_hbm, wmod_hbm,
          out_hbm, x_buf, c_buf, out_buf, ckv, wq, wuk, wuv, wo, wmod, w1, w2,
          q_lat, o_lat, words, sems):
    arrays = ([(wq_hbm, wq, 0), (wuk_hbm, wuk, 0)] + [(ckv_hbm, ckv, b * SK) for b in range(B)]
              + [(wuv_hbm, wuv, 0), (wo_hbm, wo, 0)])
    kv0, uv, ffn = 2, 2 + B, len(arrays)

    def sem(u):
        return sems.at[u % NSEM]

    def w1_group(i, g):
        cuts = [_rows(s * LANES + g * TILE, TILE) for s in range(4)]
        return [(w1_hbm.at[r, pl.ds(i * FHALF, FHALF)], w1[i].at[r], sem(ffn + i)) for r in cuts]

    def w2_group(i, g):
        size = PIECE // M
        n = 4 // len(W2_CHUNKS[i])
        return [(w2_hbm.at[_rows(f0 + (g * n + s) * size, size)],
                 w2[i].at[_rows(k * W2_ROWS + (g * n + s) * size, size)], sem(ffn + 2 + i))
                for k, f0 in enumerate(W2_CHUNKS[i]) for s in range(n)]

    ffn_runs = [
        (4, lambda g: w1_group(0, g), lambda g: w1_group(0, 4 + g)),
        (5, lambda g: w1_group(1, g), lambda g: w2_group(0, g)),
        (2, lambda g: w1_group(1, 5 + g), lambda g: w2_group(1, g)),
        (1, lambda g: w1_group(1, 7), lambda g: w2_group(2, 0)),
        (1, lambda g: w2_group(0, 5), lambda g: w2_group(2, 1)),
        (2, lambda g: w2_group(0, 6 + g), lambda g: w2_group(3, g)),
    ]

    def issue(lo, hi):
        for u, array in enumerate(arrays):
            a, b = max(lo - u * ROUNDS, 0), min(hi - u * ROUNDS, ROUNDS)
            if a < b:
                _fetch(*array, sem(u), a, b)
        r0 = ffn * ROUNDS
        for n, group0, group1 in ffn_runs:
            _loop(max(lo - r0, 0), min(hi - r0, n),
                  lambda g: _start([p for pair in zip(group0(g), group1(g)) for p in pair]))
            r0 += n

    issued = 0

    def advance(to):
        nonlocal issued
        issue(issued, to)
        issued = max(issued, to)

    def parts(u, n):
        for t in range(n):
            advance((u + 2) * ROUNDS + t * ROUNDS // n)
            if t == 0:
                _wait_filled(arrays[u][1], sem(u))
            yield t

    def wmod_round(i):
        cuts = [(_rows(s * LANES + i * TILE, TILE), pl.ds(c0, 2 * M))
                for c0 in range(0, 6 * M, 2 * M) for s in (2, 0, 3, 1)]
        _start([(wmod_hbm.at[idx], wmod.at[idx], sem(-1)) for idx in cuts])

    small = [pltpu.make_async_copy(c_hbm, c_buf, sem(-3)),
             pltpu.make_async_copy(x_hbm, x_buf, sem(-2))]
    for cp in small:
        cp.start()
    _loop(0, LANES // TILE, wmod_round)
    advance(ROUNDS)
    for cp in small:
        cp.wait()
    _wait_filled(wmod, sem(-1))

    c = c_buf[...].astype(F32)
    mod = _mm((c * jax.nn.sigmoid(c)).astype(BF16), wmod[...])
    shift_a, scale_a, gate_a, shift_b, scale_b, gate_b = (
        mod[:, i * M:(i + 1) * M] for i in range(6))
    x = x_buf[...].astype(F32)
    h = (_layernorm(x) * (1.0 + scale_a) + shift_a).astype(BF16)

    q = 0.0
    for t in parts(0, M // LANES):
        w = jnp.concatenate(list(_per_head(wq, t, words)), axis=1)
        q += _mm(h[:, t * LANES:(t + 1) * LANES], w)
    q = q.astype(BF16)
    for t in parts(1, DC // LANES):
        for hd, w in enumerate(_per_head(wuk, t, words)):
            q_lat[t, hd * B:(hd + 1) * B, :] = _mm_nt(q[:, hd * D:(hd + 1) * D], w)

    def fetch_ahead(b, lo, hi):
        pl.when(b + 2 < B)(lambda: _fetch(ckv_hbm, ckv, (b + 2) * SK, sem(kv0 + b + 2), lo, hi))
        for u in (uv, uv + 1):
            pl.when(kv0 + b + 2 == u)(lambda: _fetch(*arrays[u], sem(u), lo, hi))

    def attend(b):
        heads = pl.ds(b, H, stride=B)
        keys = _rows(b * SK, SK)
        qb = jnp.concatenate([q_lat[t, heads, :] for t in range(DC // LANES)], axis=1)
        _wait_filled(ckv.at[keys], sem(kv0 + b))
        s = _mm_nt(qb.astype(BF16), ckv[keys, :]) * D ** -0.5
        fetch_ahead(b, 0, ROUNDS // 2)
        p = jnp.exp(s - jnp.max(s, axis=-1, keepdims=True))
        o = _mm(p.astype(BF16), ckv[keys, :]) / jnp.sum(p, axis=-1, keepdims=True)
        for t in range(DC // LANES):
            o_lat[t, heads, :] = o[:, t * LANES:(t + 1) * LANES]
        fetch_ahead(b, ROUNDS // 2, ROUNDS)

    advance((kv0 + 2) * ROUNDS)
    _loop(0, B, attend)
    issued = (uv + 2) * ROUNDS

    ctx = [0.0] * H
    for t in parts(uv, DC // LANES):
        for hd, w in enumerate(_per_head(wuv, t, words)):
            ctx[hd] += _mm(o_lat[t, hd * B:(hd + 1) * B, :].astype(BF16), w)
    ctx = jnp.concatenate(ctx, axis=1).astype(BF16)
    for _ in parts(uv + 1, 1):
        x = x + gate_a * _mm(ctx, wo[...])

    h = (_layernorm(x) * (1.0 + scale_b) + shift_b).astype(BF16)
    act = []
    for i, w in enumerate(w1):
        _wait_filled(w, sem(ffn + i))
        act.append(jnp.maximum(_mm(h, w[...]), 0.0).astype(BF16))
    act = jnp.concatenate(act, axis=1)
    y = 0.0
    for i, w in enumerate(w2):
        _wait_filled(w, sem(ffn + 2 + i))
        a = jnp.concatenate([act[:, f0:f0 + W2_ROWS] for f0 in W2_CHUNKS[i]], axis=1)
        y += _mm(a, w[...])
    out_buf[...] = (x + gate_b * y).astype(out_buf.dtype)
    out = pltpu.make_async_copy(out_buf, out_hbm, sem(0))
    out.start()
    out.wait()


def _kernel(*refs):
    pl.run_scoped(lambda sems: _body(*refs, sems), pltpu.SemaphoreType.DMA((NSEM,)))


@jax.jit
def pallas_adaLN_cond__compressed_kv_cla__dense_activation_relu__decode_kernel(
        A_x, A_c_kv, A_w_q, A_w_uk, A_w_uv, A_w_o, B_x, B_w1, B_w2, c, w_mod):
    del B_x
    vmem = pltpu.VMEM
    scratch = [
        vmem((B, M), BF16), vmem((B, M), BF16), vmem((B, M), BF16),
        vmem((B * SK, DC), BF16),
        vmem((M * H, D), BF16), vmem((DC * H, D), BF16), vmem((DC * H, D), BF16),
        vmem((H * D, M), BF16),
        vmem((M, 6 * M), BF16),
        [vmem((M, FHALF), BF16) for _ in range(2)],
        [vmem((len(chunk) * W2_ROWS, M), BF16) for chunk in W2_CHUNKS],
        vmem((DC // LANES, H * B, LANES), F32), vmem((DC // LANES, H * B, LANES), F32),
        vmem((LANES * H // 2, D), U32),
    ]
    out = pl.pallas_call(
        _kernel,
        out_shape=jax.ShapeDtypeStruct((B, M), A_x.dtype),
        in_specs=[pl.BlockSpec(memory_space=pltpu.HBM)] * 10,
        out_specs=pl.BlockSpec(memory_space=pltpu.HBM),
        scratch_shapes=scratch,
        compiler_params=pltpu.CompilerParams(vmem_limit_bytes=96 * 2**20),
    )(A_x.reshape(B, M), A_c_kv.reshape(B * SK, DC), A_w_q.reshape(M * H, D),
      A_w_uk.reshape(DC * H, D), A_w_uv.reshape(DC * H, D), A_w_o.reshape(H * D, M),
      B_w1, B_w2, c, w_mod)
    return out.reshape(B, 1, M)
```
